```python
import os as _os
_os.environ.setdefault("JAX_PLATFORMS", "cpu")
import jax
import jax.numpy as jnp

def _softmax(x, axis=-1):
    return jax.nn.softmax(x, axis=axis)
def _gelu(x):
    return jax.nn.gelu(x, approximate=True)
def _silu(x):
    return jax.nn.silu(x)
def _sigmoid(x):
    return jax.nn.sigmoid(x)
def _layernorm(x, axis=-1, eps=1e-5):
    m = jnp.mean(x, axis=axis, keepdims=True)
    v = jnp.var(x, axis=axis, keepdims=True)
    return (x - m) / jnp.sqrt(v + eps)
def _scatter_add(tgt, idx, src, axis=0):
    return tgt.at[idx].add(src)
def _segment_sum(src, seg, n):
    return jax.ops.segment_sum(src, seg, n)
class _Rng:
    def __init__(self, key):
        self._k = key
    def _next(self):
        self._k, sub = jax.random.split(self._k)
        return sub
    def normal(self, shape):
        return jax.random.normal(self._next(), shape, dtype=jnp.bfloat16)
    def randint(self, lo, hi, shape):
        return jax.random.randint(self._next(), shape, lo, hi, dtype=jnp.int32)
    def uniform(self, shape, lo=0.0, hi=1.0):
        return jax.random.uniform(self._next(), shape, jnp.bfloat16, lo, hi)
    def permutation(self, n):
        return jax.random.permutation(self._next(), n)


kernel_name = 'gated_mix__mha_block__dense_activation_mish__prompt'

def setup_inputs():
    _rng = _Rng(jax.random.key(int.from_bytes(__import__("os").urandom(4), "little")))
    _w = (lambda a: (lambda t: t.astype(jnp.bfloat16) if jnp.issubdtype(t.dtype, jnp.floating) else t)(jnp.asarray(a)))
    def _A_setup():
        B, S, D, H = 1, 2048, 640, 32
        return {
            "x": _w((lambda *s: _rng.normal(s) * 0.05)(B, S, D)),
            "wqkv": _w((lambda *s: _rng.normal(s) * 0.2)(D, 3 * D)),
            "wo": _w((lambda *s: _rng.normal(s) * 0.05)(D, D)),
        }
    _A_in = _A_setup()

    def _B_setup():
        B, S, D, F = 1, 2048, 640, 1536
        return {
            "x": _w((lambda *s: _rng.normal(s) * 0.05)(B, S, D)),
            "w1": _w((lambda *s: _rng.normal(s) * 0.8)(D, F) * (D ** -0.5)),
            "b1": _w((lambda *s: _rng.normal(s) * 0.05)(F)),
            "w2": _w((lambda *s: _rng.normal(s) * 0.05)(F, D) * (F ** -0.5)),
        }
    _B_in = _B_setup()

    return {
        "A_x": _A_in["x"],
        "A_wqkv": _A_in["wqkv"],
        "A_wo": _A_in["wo"],
        "B_x": _B_in["x"],
        "B_w1": _B_in["w1"],
        "B_b1": _B_in["b1"],
        "B_w2": _B_in["w2"],
        "gate_w": _w((lambda *s: _rng.normal(s) * 0.05)(640) * 16.0),
    }

def reference(A_x, A_wqkv, A_wo, B_x, B_w1, B_b1, B_w2, gate_w):
    def _A_ref(x, wqkv, wo):
        B, S, D = x.shape
        H = 32
        Dh = D // H
        qkv = (lambda x, *d: x.transpose(*d))((x @ wqkv).reshape(B, S, 3, H, Dh), 2, 0, 3, 1, 4)
        q, k, v = qkv[0], qkv[1], qkv[2]
        scores = jnp.einsum("bhqd,bhkd->bhqk", q, k) * (Dh ** -0.5)
        p = _softmax(scores, axis=-1)
        o = jnp.einsum("bhqk,bhkd->bhqd", p, v)
        return (lambda x, *d: x.transpose(*d))(o, 0, 2, 1, 3).reshape(B, S, D) @ wo

    def _B_ref(x, w1, b1, w2):
        h = jnp.einsum("bsd,df->bsf", x, w1) + b1
        sp = jnp.log1p(jnp.exp(-jnp.abs(h))) + jnp.where(h > 0, h, jnp.zeros_like(h))
        act = h * jnp.tanh(sp)
        return jnp.einsum("bsf,fd->bsd", act, w2)

    x = A_x
    g = _sigmoid((x * gate_w).sum(-1, keepdims=True))
    a = _A_ref(x, A_wqkv, A_wo)
    b = _B_ref(x, B_w1, B_b1, B_w2)
    return g * a + (1 - g) * b
```

```python
import functools
import math

import jax
import jax.numpy as jnp
import jax.experimental.pallas as pl
import jax.experimental.pallas.tpu as pltpu
from jax import lax

_H = 32
_DH = 20
_HPS = 4
_NSLAB = _H // _HPS
_T = 512
_VR = 32
_OR = 24
_LOG2E = math.log2(math.e)

_NT = (((1,), (1,)), ((), ()))
_TNT = (((0,), (1,)), ((), ()))
_TN = (((0,), (0,)), ((), ()))


def _slabs(y, j):
    w = _HPS * _DH
    return jnp.concatenate(
        [y[:, j * w:(j + 1) * w], jnp.zeros((y.shape[0], 128 - w), y.dtype)], axis=1)


def _kernel(x_ref, wqkv_ref, wo_ref, w1_ref, b1_ref, w2_ref, gw_ref, o_ref,
            k_scr, vt_scr, q_scr, ot_scr, wo_scr, *, S, D):
    i = pl.program_id(0)
    f32, bf16 = jnp.float32, jnp.bfloat16

    @pl.when(i == 0)
    def _prologue():
        extra = (lax.broadcasted_iota(jnp.int32, (_VR - _DH, _T), 0) == 0).astype(f32)
        for c in range(S // _T):
            rows = pl.ds(c * _T, _T)
            xc = x_ref[rows, :]
            k = jnp.dot(xc, wqkv_ref[:, D:2 * D], preferred_element_type=f32).astype(bf16)
            for j in range(_NSLAB):
                k_scr[j, rows, :] = _slabs(k, j)
            vt = lax.dot_general(wqkv_ref[:, 2 * D:], xc, _TNT, preferred_element_type=f32)
            for h in range(_H):
                vt_scr[h, :, rows] = jnp.concatenate(
                    [vt[h * _DH:(h + 1) * _DH], extra], axis=0).astype(bf16)
        wo = wo_ref[...].astype(f32)
        zpad = jnp.zeros((_OR - _DH, D), f32)
        wo_scr[...] = jnp.concatenate(
            [p for h in range(_H) for p in (wo[h * _DH:(h + 1) * _DH], zpad)], axis=0).astype(bf16)

    x = x_ref[pl.ds(pl.multiple_of(i * _T, _T), _T), :]
    q = (jnp.dot(x, wqkv_ref[:, :D], preferred_element_type=f32)
         * (_DH ** -0.5 * _LOG2E)).astype(bf16)
    for j in range(_NSLAB):
        q_scr[j] = _slabs(q, j)

    lane = lax.broadcasted_iota(jnp.int32, (_T, 128), 1)

    def head(h, carry):
        j = h // _HPS
        lo = (h % _HPS) * _DH
        qh = jnp.where((lane >= lo) & (lane < lo + _DH), q_scr[j].astype(f32), 0.0).astype(bf16)
        st = lax.dot_general(k_scr[j], qh, _NT, preferred_element_type=f32)
        p = jnp.exp2(st - jnp.max(st, axis=0, keepdims=True)).astype(bf16)
        ot = jnp.dot(vt_scr[h], p, preferred_element_type=f32)
        ot_scr[pl.ds(pl.multiple_of(h * _OR, 8), _OR), :] = ot[:_OR] / ot[_DH:_DH + 1]
        return carry

    lax.fori_loop(0, _H, head, 0)

    a = lax.dot_general(ot_scr[...].astype(bf16), wo_scr[...], _TN, preferred_element_type=f32)

    hid = jnp.dot(x, w1_ref[...], preferred_element_type=f32) + b1_ref[...].astype(f32)
    e = jnp.exp(jnp.minimum(hid, 20.0))
    n = e * (e + 2.0)
    act = (hid * (n / (n + 2.0))).astype(bf16)
    b = jnp.dot(act, w2_ref[...], preferred_element_type=f32)

    g = jax.nn.sigmoid(jnp.sum(x.astype(f32) * gw_ref[...].astype(f32), axis=-1, keepdims=True))
    o_ref[...] = (g * a + (1.0 - g) * b).astype(o_ref.dtype)


@jax.jit
def pallas_gated_mix__mha_block__dense_activation_mish__prompt_kernel(
    A_x: jax.Array,
    A_wqkv: jax.Array,
    A_wo: jax.Array,
    B_x: jax.Array,
    B_w1: jax.Array,
    B_b1: jax.Array,
    B_w2: jax.Array,
    gate_w: jax.Array,
):
    del B_x
    B, S, D = A_x.shape
    F = B_w1.shape[1]
    whole = lambda shape: pl.BlockSpec(shape, lambda i: (0,) * len(shape))
    out = pl.pallas_call(
        functools.partial(_kernel, S=S, D=D),
        grid=(S // _T,),
        in_specs=[whole((S, D)), whole((D, 3 * D)), whole((D, D)), whole((D, F)),
                  whole((1, F)), whole((F, D)), whole((1, D))],
        out_specs=pl.BlockSpec((_T, D), lambda i: (i, 0)),
        out_shape=jax.ShapeDtypeStruct((S, D), A_x.dtype),
        scratch_shapes=[
            pltpu.VMEM((_NSLAB, S, 128), jnp.bfloat16),
            pltpu.VMEM((_H, _VR, S), jnp.bfloat16),
            pltpu.VMEM((_NSLAB, _T, 128), jnp.bfloat16),
            pltpu.VMEM((_H * _OR, _T), jnp.float32),
            pltpu.VMEM((_H * _OR, D), jnp.bfloat16),
        ],
        compiler_params=pltpu.CompilerParams(
            dimension_semantics=("arbitrary",),
            vmem_limit_bytes=100 * 1024 * 1024,
        ),
    )(A_x.reshape(S, D), A_wqkv, A_wo, B_w1, B_b1.reshape(1, F), B_w2, gate_w.reshape(1, D))
    return out.reshape(B, S, D)
```

```python
import functools
import math

import jax
import jax.numpy as jnp
import jax.experimental.pallas as pl
import jax.experimental.pallas.tpu as pltpu
from jax import lax

_H = 32
_DH = 20
_HPS = 4
_NSLAB = _H // _HPS
_T = 512
_C = 128
_VR = 24
_FP = 256
_QSCALE = _DH ** -0.5 * math.log2(math.e)

_NN = (((1,), (0,)), ((), ()))
_NT = (((1,), (1,)), ((), ()))
_TN = (((0,), (0,)), ((), ()))
_TT = (((0,), (1,)), ((), ()))


def _slab(y, j):
    w = _HPS * _DH
    return jnp.concatenate(
        [y[:, j * w:(j + 1) * w], jnp.zeros((y.shape[0], 128 - w), y.dtype)], axis=1)


def _mish(h):
    e = jnp.exp(jnp.minimum(h, 20.0))
    n = e * (e + 2.0)
    return (h * (n / (n + 2.0))).astype(jnp.bfloat16)


def _kernel(x_hbm, wqkv_hbm, wo_hbm, w1_hbm, b1_hbm, w2_hbm, gw_hbm, o_hbm,
            x_ref, wq_ref, wkv_ref, wo_ref, w1_ref, w2_ref, o_scr,
            k_scr, vt_scr, q_scr, ot_scr, s_scr, m_scr, b1_ref, gw_ref,
            xsem, wsem, osem, *, S, D):
    f32, bf16 = jnp.float32, jnp.bfloat16
    NQ = S // _T
    NC = S // _C
    LNS = _NSLAB.bit_length() - 1

    def tile(c):
        return pl.ds(pl.multiple_of(c * _T, _T), _T)

    def x_copy(c):
        return pltpu.make_async_copy(x_hbm.at[0, tile(c), :], x_ref.at[tile(c), :], xsem.at[c])

    def o_copy(c):
        return pltpu.make_async_copy(o_scr.at[tile(c), :], o_hbm.at[0, tile(c), :], osem.at[c])

    wq_copy = pltpu.make_async_copy(wqkv_hbm.at[:, pl.ds(0, D)], wq_ref, wsem.at[0])
    wkv_copy = pltpu.make_async_copy(wqkv_hbm.at[:, pl.ds(D, 2 * D)], wkv_ref, wsem.at[1])
    late_copies = [
        pltpu.make_async_copy(wo_hbm, wo_ref, wsem.at[2]),
        pltpu.make_async_copy(w1_hbm, w1_ref, wsem.at[3]),
        pltpu.make_async_copy(b1_hbm, b1_ref, wsem.at[4]),
        pltpu.make_async_copy(w2_hbm, w2_ref, wsem.at[5]),
        pltpu.make_async_copy(gw_hbm, gw_ref, wsem.at[6]),
    ]

    x_copy(0).start()
    wq_copy.start()
    x_copy(0).wait()
    wq_copy.wait()
    for c in range(1, NQ):
        x_copy(c).start()
    wkv_copy.start()

    def proj_q(c, carry):
        @pl.when(c >= 1)
        def _():
            x_copy(c).wait()

        q = (jnp.dot(x_ref[tile(c), :], wq_ref[...], preferred_element_type=f32)
             * _QSCALE).astype(bf16)
        for j in range(_NSLAB):
            q_scr[j, tile(c), :] = _slab(q, j)
        return carry

    lax.fori_loop(0, NQ, proj_q, 0)
    wkv_copy.wait()
    for cp in late_copies:
        cp.start()

    ones_rows = (lax.broadcasted_iota(jnp.int32, (_VR - _DH, _T), 0) == 0).astype(f32)

    def proj_kv(c, carry):
        xc = x_ref[tile(c), :]
        k = jnp.dot(xc, wkv_ref[:, :D], preferred_element_type=f32).astype(bf16)
        half = pl.ds(pl.multiple_of(c * (_T // 2), _T // 2), _T // 2)
        for j in range(_NSLAB):
            k_scr[j, half, :] = pltpu.bitcast(_slab(k, j), jnp.int32)
        vt = lax.dot_general(wkv_ref[:, D:], xc, _TT, preferred_element_type=f32)
        vt = vt.astype(bf16).astype(f32)
        for h in range(_H):
            vt_scr[h, :, tile(c)] = jnp.concatenate(
                [vt[h * _DH:(h + 1) * _DH], ones_rows], axis=0)
        return carry

    lax.fori_loop(0, NQ, proj_kv, 0)

    lane = lax.broadcasted_iota(jnp.int32, (_T, 128), 1)

    def group(t, scores=True, softmax=True, hook=None):
        if scores:
            qa, ja = (t + 1) >> LNS, (t + 1) & (_NSLAB - 1)
        if softmax:
            qb, jb = t >> LNS, t & (_NSLAB - 1)
            outs = []
        for i in range(_HPS):
            if scores:
                mine = (lane >= i * _DH) & (lane < (i + 1) * _DH)
                qh = jnp.where(mine, q_scr[ja, tile(qa), :].astype(f32), 0.0).astype(bf16)
                m8 = jnp.full((8, _T), -jnp.inf, f32)
            if softmax:
                m = jnp.max(m_scr[8 * i:8 * i + 8, :], axis=0, keepdims=True)
                acc = jnp.zeros((_VR, _T), f32)
            for c in range(NC):
                rows = pl.ds(c * _C, _C)
                if softmax:
                    p = jnp.exp2(s_scr[i, rows, :] - m).astype(bf16)
                    acc = acc + lax.dot_general(
                        vt_scr[jb * _HPS + i, :, rows], p, _NN, preferred_element_type=f32)
                if scores:
                    kc = pltpu.bitcast(k_scr[ja, pl.ds(c * _C // 2, _C // 2), :], bf16)
                    s = lax.dot_general(kc, qh, _NT, preferred_element_type=f32)
                    s_scr[i, rows, :] = s
                    m8 = jnp.maximum(m8, jnp.max(s.reshape(_C // 8, 8, _T), axis=0))
                if hook is not None:
                    hook(i * NC + c)
            if scores:
                m_scr[8 * i:8 * i + 8, :] = m8
            if softmax:
                outs.append(acc[:_DH] / acc[_DH:_DH + 1])
        if softmax:
            w = _HPS * _DH
            ot_scr[pl.ds(pl.multiple_of(jb * w, 16), w), tile(qb)] = (
                jnp.concatenate(outs, axis=0).astype(bf16))

    group(jnp.int32(-1), softmax=False)

    def body(t, carry):
        group(t)
        return carry

    lax.fori_loop(0, NQ * _NSLAB - 1, body, 0)

    for cp in late_copies:
        cp.wait()

    def finish(c, x, b):
        a = lax.dot_general(ot_scr[:, tile(c)], wo_ref[...], _TN, preferred_element_type=f32)
        g = jax.nn.sigmoid(jnp.sum(
            x.astype(f32) * gw_ref[...].astype(f32)[None, :], axis=-1, keepdims=True))
        o_scr[tile(c), :] = (g * a + (1.0 - g) * b).astype(o_scr.dtype)
        o_copy(c).start()

    x0 = x_ref[pl.ds(0, _T), :]
    b1 = b1_ref[...].astype(f32)[None, :]
    n_pieces = w1_ref.shape[1] // _FP
    every = _HPS * NC // (2 * n_pieces)
    st = {}

    def ffn_hook(k):
        u, r = divmod(k + 1, every)
        if r or u > 2 * n_pieces:
            return
        p, second = divmod(u - 1, 2)
        cols = slice(p * _FP, (p + 1) * _FP)
        if second:
            d = jnp.dot(st["act"], w2_ref[cols, :], preferred_element_type=f32)
            st["b"] = d if p == 0 else st["b"] + d
        else:
            st["act"] = _mish(
                jnp.dot(x0, w1_ref[:, cols], preferred_element_type=f32) + b1[:, cols])

    group(jnp.int32(NQ * _NSLAB - 1), scores=False, hook=ffn_hook)
    finish(0, x0, st["b"])

    def epilogue(c, carry):
        x = x_ref[tile(c), :]
        h = jnp.dot(x, w1_ref[...], preferred_element_type=f32) + b1_ref[...].astype(f32)[None, :]
        finish(c, x, jnp.dot(_mish(h), w2_ref[...], preferred_element_type=f32))
        return carry

    lax.fori_loop(1, NQ, epilogue, 0)
    for c in range(NQ):
        o_copy(c).wait()


@jax.jit
def pallas_gated_mix__mha_block__dense_activation_mish__prompt_kernel(
    A_x: jax.Array,
    A_wqkv: jax.Array,
    A_wo: jax.Array,
    B_x: jax.Array,
    B_w1: jax.Array,
    B_b1: jax.Array,
    B_w2: jax.Array,
    gate_w: jax.Array,
):
    del B_x
    B, S, D = A_x.shape
    F = B_w1.shape[1]
    bf16, f32 = jnp.bfloat16, jnp.float32
    return pl.pallas_call(
        functools.partial(_kernel, S=S, D=D),
        out_shape=jax.ShapeDtypeStruct((B, S, D), A_x.dtype),
        in_specs=[pl.BlockSpec(memory_space=pl.ANY)] * 7,
        out_specs=pl.BlockSpec(memory_space=pl.ANY),
        scratch_shapes=[
            pltpu.VMEM((S, D), bf16),
            pltpu.VMEM((D, D), bf16),
            pltpu.VMEM((D, 2 * D), bf16),
            pltpu.VMEM((D, D), bf16),
            pltpu.VMEM((D, F), bf16),
            pltpu.VMEM((F, D), bf16),
            pltpu.VMEM((S, D), bf16),
            pltpu.VMEM((_NSLAB, S // 2, 128), jnp.int32),
            pltpu.VMEM((_H, _VR, S), f32),
            pltpu.VMEM((_NSLAB, S, 128), bf16),
            pltpu.VMEM((D, S), bf16),
            pltpu.VMEM((_HPS, S, _T), f32),
            pltpu.VMEM((_HPS * 8, _T), f32),
            pltpu.VMEM((F,), bf16),
            pltpu.VMEM((D,), bf16),
            pltpu.SemaphoreType.DMA((S // _T,)),
            pltpu.SemaphoreType.DMA((7,)),
            pltpu.SemaphoreType.DMA((S // _T,)),
        ],
        compiler_params=pltpu.CompilerParams(vmem_limit_bytes=100 * 1024 * 1024),
    )(A_x, A_wqkv, A_wo, B_w1, B_b1, B_w2, gate_w)
```

```python
import functools
import math

import jax
import jax.numpy as jnp
import jax.experimental.pallas as pl
import jax.experimental.pallas.tpu as pltpu
from jax import lax

_H = 32
_DH = 20
_HPS = 4
_NSLAB = _H // _HPS
_T = 512
_C = 128
_VR = 24
_FP = 256
_QSCALE = _DH ** -0.5 * math.log2(math.e)

_NN = (((1,), (0,)), ((), ()))
_NT = (((1,), (1,)), ((), ()))
_TN = (((0,), (0,)), ((), ()))
_TT = (((0,), (1,)), ((), ()))


def _slab(y, j):
    w = _HPS * _DH
    return jnp.concatenate(
        [y[:, j * w:(j + 1) * w], jnp.zeros((y.shape[0], 128 - w), y.dtype)], axis=1)


def _mish(h):
    e = jnp.exp(jnp.minimum(h, 20.0))
    n = e * (e + 2.0)
    return (h * (n / (n + 2.0))).astype(jnp.bfloat16)


def _kernel(x_hbm, wqkv_hbm, wo_hbm, w1_hbm, b1_hbm, w2_hbm, gw_hbm, o_hbm,
            x_ref, wq_ref, wkv_ref, wo_ref, w1_ref, w2_ref, o_scr,
            k_scr, vt_scr, q_scr, ot_scr, s_scr, m_scr, b1_ref, gw_ref,
            xsem, wsem, osem, *, S, D):
    f32, bf16 = jnp.float32, jnp.bfloat16
    NQ = S // _T
    NC = S // _C
    LNS = _NSLAB.bit_length() - 1

    def tile(c):
        return pl.ds(pl.multiple_of(c * _T, _T), _T)

    def x_copy(c):
        return pltpu.make_async_copy(x_hbm.at[0, tile(c), :], x_ref.at[tile(c), :], xsem.at[c])

    def o_copy(c):
        return pltpu.make_async_copy(o_scr.at[tile(c), :], o_hbm.at[0, tile(c), :], osem.at[c])

    wq_copy = pltpu.make_async_copy(wqkv_hbm.at[:, pl.ds(0, D)], wq_ref, wsem.at[0])
    wkv_copy = pltpu.make_async_copy(wqkv_hbm.at[:, pl.ds(D, 2 * D)], wkv_ref, wsem.at[1])
    late_copies = [
        pltpu.make_async_copy(wo_hbm, wo_ref, wsem.at[2]),
        pltpu.make_async_copy(w1_hbm, w1_ref, wsem.at[3]),
        pltpu.make_async_copy(b1_hbm, b1_ref, wsem.at[4]),
        pltpu.make_async_copy(w2_hbm, w2_ref, wsem.at[5]),
        pltpu.make_async_copy(gw_hbm, gw_ref, wsem.at[6]),
    ]

    x_copy(0).start()
    wq_copy.start()
    x_copy(0).wait()
    wq_copy.wait()
    for c in range(1, NQ):
        x_copy(c).start()
    wkv_copy.start()

    def proj_q(c, carry):
        @pl.when(c >= 1)
        def _():
            x_copy(c).wait()

        q = (jnp.dot(x_ref[tile(c), :], wq_ref[...], preferred_element_type=f32)
             * _QSCALE).astype(bf16)
        for j in range(_NSLAB):
            q_scr[j, tile(c), :] = _slab(q, j)
        return carry

    lax.fori_loop(0, NQ, proj_q, 0)
    wkv_copy.wait()
    for cp in late_copies:
        cp.start()

    ones_rows = (lax.broadcasted_iota(jnp.int32, (_VR - _DH, _T), 0) == 0).astype(f32)

    def proj_kv(c, carry):
        xc = x_ref[tile(c), :]
        k = jnp.dot(xc, wkv_ref[:, :D], preferred_element_type=f32).astype(bf16)
        half = pl.ds(pl.multiple_of(c * (_T // 2), _T // 2), _T // 2)
        for j in range(_NSLAB):
            k_scr[j, half, :] = pltpu.bitcast(_slab(k, j), jnp.int32)
        vt = lax.dot_general(wkv_ref[:, D:], xc, _TT, preferred_element_type=f32)
        vt = vt.astype(bf16).astype(f32)
        for h in range(_H):
            vt_scr[h, :, tile(c)] = jnp.concatenate(
                [vt[h * _DH:(h + 1) * _DH], ones_rows], axis=0)
        return carry

    lax.fori_loop(0, NQ, proj_kv, 0)

    lane = lax.broadcasted_iota(jnp.int32, (_T, 128), 1)

    def group(t, scores=True, softmax=True, hook=None):
        if scores:
            qa, ja = (t + 1) >> LNS, (t + 1) & (_NSLAB - 1)
        if softmax:
            qb, jb = t >> LNS, t & (_NSLAB - 1)
            outs = []
        for i in range(_HPS):
            if scores:
                mine = (lane >= i * _DH) & (lane < (i + 1) * _DH)
                qh = jnp.where(mine, q_scr[ja, tile(qa), :].astype(f32), 0.0).astype(bf16)
                m8 = jnp.full((8, _T), -jnp.inf, f32)
            if softmax:
                m = jnp.max(m_scr[8 * i:8 * i + 8, :], axis=0, keepdims=True)
                acc = jnp.zeros((_VR, _T), f32)
            for c in range(NC):
                rows = pl.ds(c * _C, _C)
                if softmax:
                    p = jnp.exp2(s_scr[i, rows, :] - m).astype(bf16)
                    acc = acc + lax.dot_general(
                        vt_scr[jb * _HPS + i, :, rows], p, _NN, preferred_element_type=f32)
                if scores:
                    kc = pltpu.bitcast(k_scr[ja, pl.ds(c * _C // 2, _C // 2), :], bf16)
                    s = lax.dot_general(kc, qh, _NT, preferred_element_type=f32)
                    s_scr[i, rows, :] = s
                    m8 = jnp.maximum(m8, jnp.max(s.reshape(_C // 8, 8, _T), axis=0))
                if hook is not None:
                    hook(i * NC + c)
            if scores:
                m_scr[8 * i:8 * i + 8, :] = m8
            if softmax:
                outs.append(acc[:_DH] / acc[_DH:_DH + 1])
        if softmax:
            w = _HPS * _DH
            ot_scr[pl.ds(pl.multiple_of(jb * w, 16), w), tile(qb)] = (
                jnp.concatenate(outs, axis=0).astype(bf16))

    group(jnp.int32(-1), softmax=False)

    def body(u, carry):
        group(2 * u + 1)
        group(2 * u + 2)
        return carry

    group(jnp.int32(0))
    lax.fori_loop(0, NQ * _NSLAB // 2 - 1, body, 0)

    for cp in late_copies:
        cp.wait()

    def finish(c, x, b):
        a = lax.dot_general(ot_scr[:, tile(c)], wo_ref[...], _TN, preferred_element_type=f32)
        g = jax.nn.sigmoid(jnp.sum(
            x.astype(f32) * gw_ref[...].astype(f32)[None, :], axis=-1, keepdims=True))
        o_scr[tile(c), :] = (g * a + (1.0 - g) * b).astype(o_scr.dtype)
        o_copy(c).start()

    x0 = x_ref[pl.ds(0, _T), :]
    b1 = b1_ref[...].astype(f32)[None, :]
    n_pieces = w1_ref.shape[1] // _FP
    every = _HPS * NC // (2 * n_pieces)
    st = {}

    def ffn_hook(k):
        u, r = divmod(k + 1, every)
        if r or u > 2 * n_pieces:
            return
        p, second = divmod(u - 1, 2)
        cols = slice(p * _FP, (p + 1) * _FP)
        if second:
            d = jnp.dot(st["act"], w2_ref[cols, :], preferred_element_type=f32)
            st["b"] = d if p == 0 else st["b"] + d
        else:
            st["act"] = _mish(
                jnp.dot(x0, w1_ref[:, cols], preferred_element_type=f32) + b1[:, cols])

    group(jnp.int32(NQ * _NSLAB - 1), scores=False, hook=ffn_hook)
    finish(0, x0, st["b"])

    def epilogue(c, carry):
        x = x_ref[tile(c), :]
        h = jnp.dot(x, w1_ref[...], preferred_element_type=f32) + b1_ref[...].astype(f32)[None, :]
        finish(c, x, jnp.dot(_mish(h), w2_ref[...], preferred_element_type=f32))
        return carry

    lax.fori_loop(1, NQ, epilogue, 0)
    for c in range(NQ):
        o_copy(c).wait()


@jax.jit
def pallas_gated_mix__mha_block__dense_activation_mish__prompt_kernel(
    A_x: jax.Array,
    A_wqkv: jax.Array,
    A_wo: jax.Array,
    B_x: jax.Array,
    B_w1: jax.Array,
    B_b1: jax.Array,
    B_w2: jax.Array,
    gate_w: jax.Array,
):
    del B_x
    B, S, D = A_x.shape
    F = B_w1.shape[1]
    bf16, f32 = jnp.bfloat16, jnp.float32
    return pl.pallas_call(
        functools.partial(_kernel, S=S, D=D),
        out_shape=jax.ShapeDtypeStruct((B, S, D), A_x.dtype),
        in_specs=[pl.BlockSpec(memory_space=pl.ANY)] * 7,
        out_specs=pl.BlockSpec(memory_space=pl.ANY),
        scratch_shapes=[
            pltpu.VMEM((S, D), bf16),
            pltpu.VMEM((D, D), bf16),
            pltpu.VMEM((D, 2 * D), bf16),
            pltpu.VMEM((D, D), bf16),
            pltpu.VMEM((D, F), bf16),
            pltpu.VMEM((F, D), bf16),
            pltpu.VMEM((S, D), bf16),
            pltpu.VMEM((_NSLAB, S // 2, 128), jnp.int32),
            pltpu.VMEM((_H, _VR, S), f32),
            pltpu.VMEM((_NSLAB, S, 128), bf16),
            pltpu.VMEM((D, S), bf16),
            pltpu.VMEM((_HPS, S, _T), f32),
            pltpu.VMEM((_HPS * 8, _T), f32),
            pltpu.VMEM((F,), bf16),
            pltpu.VMEM((D,), bf16),
            pltpu.SemaphoreType.DMA((S // _T,)),
            pltpu.SemaphoreType.DMA((7,)),
            pltpu.SemaphoreType.DMA((S // _T,)),
        ],
        compiler_params=pltpu.CompilerParams(vmem_limit_bytes=100 * 1024 * 1024),
    )(A_x, A_wqkv, A_wo, B_w1, B_b1, B_w2, gate_w)
```
